```python
import os as _os
_os.environ.setdefault('JAX_PLATFORMS', 'cpu')
import jax
import jax.numpy as jnp

def _softmax(x, axis=-1):
    return jax.nn.softmax(x, axis=axis)

def _gelu(x):
    return jax.nn.gelu(x, approximate=True)

def _silu(x):
    return jax.nn.silu(x)

def _sigmoid(x):
    return jax.nn.sigmoid(x)

def _layernorm(x, axis=-1, eps=1e-05):
    m = jnp.mean(x, axis=axis, keepdims=True)
    v = jnp.var(x, axis=axis, keepdims=True)
    return (x - m) / jnp.sqrt(v + eps)

def _scatter_add(tgt, idx, src, axis=0):
    return tgt.at[idx].add(src)

def _segment_sum(src, seg, n):
    return jax.ops.segment_sum(src, seg, n)

class _Rng:

    def __init__(self, key):
        self._k = key

    def _next(self):
        self._k, sub = jax.random.split(self._k)
        return sub

    def normal(self, shape):
        return jax.random.normal(self._next(), shape, dtype=jnp.bfloat16)

    def randint(self, lo, hi, shape):
        return jax.random.randint(self._next(), shape, lo, hi, dtype=jnp.int32)

    def uniform(self, shape, lo=0.0, hi=1.0):
        return jax.random.uniform(self._next(), shape, jnp.bfloat16, lo, hi)

    def permutation(self, n):
        return jax.random.permutation(self._next(), n)
kernel_name = 'sequential_preLN__linear_attn_block__mixer_gmlp__prompt'

def setup_inputs():
    _rng = _Rng(jax.random.key(int.from_bytes(__import__("os").urandom(4), "little")))
    _w = lambda a: (lambda t: t.astype(jnp.bfloat16) if jnp.issubdtype(t.dtype, jnp.floating) else t)(jnp.asarray(a))

    def _A_setup():
        B, S, D = (1, 2048, 512)
        return {'x': _w((lambda *s: _rng.normal(s) * 0.05)(B, S, D)), 'wqkv': _w((lambda *s: _rng.normal(s) * 0.05)(D, 3 * D)), 'wo': _w((lambda *s: _rng.normal(s) * 0.05)(D, D))}
    _A_in = _A_setup()

    def _B_setup():
        B, S, D, F = (1, 2048, 512, 1792)
        Fh = F // 2
        return {'x': _w((lambda *s: _rng.normal(s) * 0.05)(B, S, D)), 'w_in': _w((lambda *s: _rng.normal(s) * 0.4)(D, 2 * Fh)), 'w_sp': _w(0.01 * (lambda *s: _rng.normal(s) * 0.4)(S, S)), 'b_sp': _w(1.0 + 0.01 * (lambda *s: _rng.normal(s) * 0.05)(S)), 'w_out': _w((lambda *s: _rng.normal(s) * 0.05)(Fh, D))}
    _B_in = _B_setup()
    return {'A_x': _A_in['x'], 'A_wqkv': _A_in['wqkv'], 'A_wo': _A_in['wo'], 'B_x': _B_in['x'], 'B_w_in': _B_in['w_in'], 'B_w_sp': _B_in['w_sp'], 'B_b_sp': _B_in['b_sp'], 'B_w_out': _B_in['w_out']}

def reference(A_x, A_wqkv, A_wo, B_x, B_w_in, B_w_sp, B_b_sp, B_w_out):

    def _A_ref(x, wqkv, wo):
        B, S, D = x.shape
        H = 32
        Dh = D // H
        qkv = (lambda x, *d: x.transpose(*d))((x @ wqkv).reshape(B, S, 3, H, Dh), 2, 0, 3, 1, 4)
        q, k, v = (qkv[0], qkv[1], qkv[2])
        phi = lambda t: jnp.where(t > 0, t + 1, jnp.exp(t)) + 1e-06
        pq, pk = (phi(q), phi(k))
        kv = jnp.einsum('bhsd,bhse->bhde', pk, v)
        z = jnp.einsum('bhsd->bhd', pk)
        num = jnp.einsum('bhqd,bhde->bhqe', pq, kv)
        den = jnp.einsum('bhqd,bhd->bhq', pq, z)[..., None] + 1e-06
        o = num / den
        return (lambda x, *d: x.transpose(*d))(o, 0, 2, 1, 3).reshape(B, S, D) @ wo

    def _B_ref(x, w_in, w_sp, b_sp, w_out):
        B, S, D = x.shape
        F = w_in.shape[-1]
        Fh = F // 2
        z = _gelu(jnp.einsum('bsd,df->bsf', x, w_in))
        z1 = z[..., :Fh].copy()
        z2 = _layernorm(z[..., Fh:], axis=-1)
        g = jnp.einsum('ts,bsf->btf', w_sp, z2) + b_sp[None, :, None]
        return jnp.einsum('bsf,fd->bsd', z1 * g, w_out)
    x = A_x
    h = x + _A_ref(_layernorm(x, axis=-1), A_wqkv, A_wo)
    h2 = h + _B_ref(_layernorm(h, axis=-1), B_w_in, B_w_sp, B_b_sp, B_w_out)
    return h2
```

```python
import functools
import jax
import jax.numpy as jnp
from jax import lax
import jax.experimental.pallas as pl
import jax.experimental.pallas.tpu as pltpu

S = 2048
D = 512
FH = 896
DH = 16
TM1 = 256
TM2 = 256
TM3 = 256
F32 = jnp.float32
BF16 = jnp.bfloat16


def _ln(x):
    m = jnp.mean(x, axis=-1, keepdims=True)
    xc = x - m
    v = jnp.mean(xc * xc, axis=-1, keepdims=True)
    return xc * lax.rsqrt(v + 1e-5)


def _phi(t):
    return jnp.where(t > 0, t + 1.0, jnp.exp(t)) + 1e-6


def _kernel(x_hbm, wqkv_hbm, wo_hbm, win_hbm, wsp_hbm, b_hbm, wout_hbm, out_hbm,
            x_v, wqkv_v, wo_v, win_v, wsp_v, b_v, wout_v, out_v,
            pq_s, h_s, z1_s, z2_s, kv_s, zs_s, zb_s, kvwo_s, bcol_s, sems, osems):
    c_x = pltpu.make_async_copy(x_hbm, x_v, sems.at[0])
    c_wqkv = pltpu.make_async_copy(wqkv_hbm, wqkv_v, sems.at[1])
    c_wo = pltpu.make_async_copy(wo_hbm, wo_v, sems.at[2])
    c_win = pltpu.make_async_copy(win_hbm, win_v, sems.at[3])
    c_wsp = pltpu.make_async_copy(wsp_hbm, wsp_v, sems.at[4])
    c_b = pltpu.make_async_copy(b_hbm, b_v, sems.at[5])
    c_wout = pltpu.make_async_copy(wout_hbm, wout_v, sems.at[6])
    c_x.start()
    c_wqkv.start()
    c_x.wait()
    c_wqkv.wait()
    c_wo.start()
    c_win.start()
    c_b.start()
    c_wout.start()
    c_wsp.start()

    kv_s[...] = jnp.zeros_like(kv_s)
    zs_s[...] = jnp.zeros_like(zs_s)

    def p1(i, c):
        r = pl.multiple_of(i * TM1, TM1)
        x = x_v[pl.ds(r, TM1), :].astype(F32)
        xn = _ln(x).astype(BF16)
        qkv = jnp.dot(xn, wqkv_v[...], preferred_element_type=F32)
        pq = _phi(qkv[:, :D])
        pk = _phi(qkv[:, D:2 * D])
        v = qkv[:, 2 * D:].astype(BF16)
        pq_s[pl.ds(r, TM1), :] = pq.astype(BF16)
        zs_s[...] += jnp.sum(pk, axis=0, keepdims=True)
        pkb = pk.astype(BF16)
        for j in range(4):
            kv_s[j] += lax.dot_general(
                pkb[:, j * 128:(j + 1) * 128], v[:, j * 128:(j + 1) * 128],
                (((0,), (0,)), ((), ())), preferred_element_type=F32)
        return c

    lax.fori_loop(0, S // TM1, p1, 0)

    c_wo.wait()
    c_b.wait()
    rr = lax.broadcasted_iota(jnp.int32, (128, 128), 0) // DH
    cc = lax.broadcasted_iota(jnp.int32, (128, 128), 1) // DH
    mask = rr == cc
    for j in range(4):
        kvm = jnp.where(mask, kv_s[j], 0.0).astype(BF16)
        kvwo_s[j * 128:(j + 1) * 128, :] = jnp.dot(
            kvm, wo_v[j * 128:(j + 1) * 128, :], preferred_element_type=F32).astype(BF16)
        zrow = jnp.broadcast_to(zs_s[:, j * 128:(j + 1) * 128], (128, 128))
        zb_s[j] = jnp.where(mask, zrow.T, 0.0).astype(BF16)
    bb = b_v[...].astype(F32)
    for j in range(16):
        bcol_s[j * 128:(j + 1) * 128, :] = jnp.broadcast_to(bb[j:j + 1, :], (128, 128)).T

    c_win.wait()

    def p2(i, c):
        r = pl.multiple_of(i * TM2, TM2)
        pq = pq_s[pl.ds(r, TM2), :]
        den = jnp.concatenate(
            [jnp.dot(pq[:, j * 128:(j + 1) * 128], zb_s[j], preferred_element_type=F32)
             for j in range(4)], axis=1) + 1e-6
        a = (pq.astype(F32) / den).astype(BF16)
        h = x_v[pl.ds(r, TM2), :].astype(F32) + jnp.dot(a, kvwo_s[...], preferred_element_type=F32)
        h_s[pl.ds(r, TM2), :] = h
        hn = _ln(h).astype(BF16)
        zz = jax.nn.gelu(jnp.dot(hn, win_v[...], preferred_element_type=F32), approximate=True)
        z1_s[pl.ds(r, TM2), :] = zz[:, :FH]
        z2_s[pl.ds(r, TM2), :] = _ln(zz[:, FH:]).astype(BF16)
        return c

    lax.fori_loop(0, S // TM2, p2, 0)

    c_wsp.wait()
    c_wout.wait()

    def out_copy(i):
        r = pl.multiple_of(i * TM3, TM3)
        return pltpu.make_async_copy(out_v.at[pl.ds(r, TM3), :], out_hbm.at[pl.ds(r, TM3), :], osems.at[i])

    def p3(i, c):
        r = pl.multiple_of(i * TM3, TM3)
        g = jnp.dot(wsp_v[pl.ds(r, TM3), :], z2_s[...], preferred_element_type=F32)
        bc = bcol_s[pl.ds(r, TM3), :]
        g = g + jnp.concatenate([bc] * (FH // 128), axis=1)
        u = (z1_s[pl.ds(r, TM3), :] * g).astype(BF16)
        o = h_s[pl.ds(r, TM3), :] + jnp.dot(u, wout_v[...], preferred_element_type=F32)
        out_v[pl.ds(r, TM3), :] = o.astype(BF16)
        out_copy(i).start()
        return c

    lax.fori_loop(0, S // TM3, p3, 0)
    for i in range(S // TM3):
        out_copy(i).wait()


@jax.jit
def pallas_sequential_preLN__linear_attn_block__mixer_gmlp__prompt_kernel(
    A_x, A_wqkv, A_wo, B_x, B_w_in, B_w_sp, B_b_sp, B_w_out):
    x = A_x.reshape(S, D)
    b2 = B_b_sp.reshape(S // 128, 128)
    any_spec = pl.BlockSpec(memory_space=pl.ANY)
    out = pl.pallas_call(
        _kernel,
        out_shape=jax.ShapeDtypeStruct((S, D), BF16),
        in_specs=[any_spec] * 7,
        out_specs=any_spec,
        scratch_shapes=[
            pltpu.VMEM((S, D), BF16),
            pltpu.VMEM((D, 3 * D), BF16),
            pltpu.VMEM((D, D), BF16),
            pltpu.VMEM((D, 2 * FH), BF16),
            pltpu.VMEM((S, S), BF16),
            pltpu.VMEM((S // 128, 128), BF16),
            pltpu.VMEM((FH, D), BF16),
            pltpu.VMEM((S, D), BF16),
            pltpu.VMEM((S, D), BF16),
            pltpu.VMEM((S, D), F32),
            pltpu.VMEM((S, FH), F32),
            pltpu.VMEM((S, FH), BF16),
            pltpu.VMEM((4, 128, 128), F32),
            pltpu.VMEM((1, D), F32),
            pltpu.VMEM((4, 128, 128), BF16),
            pltpu.VMEM((D, D), BF16),
            pltpu.VMEM((S, 128), F32),
            pltpu.SemaphoreType.DMA((7,)),
            pltpu.SemaphoreType.DMA((S // TM3,)),
        ],
        compiler_params=pltpu.CompilerParams(vmem_limit_bytes=100 * 1024 * 1024),
    )(x, A_wqkv, A_wo, B_w_in, B_w_sp, b2, B_w_out)
    return out.reshape(1, S, D)
```

```python
import functools
import jax
import jax.numpy as jnp
from jax import lax
import jax.experimental.pallas as pl
import jax.experimental.pallas.tpu as pltpu

S = 2048
D = 512
FH = 896
DH = 16
TM = 256
NB = S // TM
F32 = jnp.float32
BF16 = jnp.bfloat16


def _ln(x):
    m = jnp.mean(x, axis=-1, keepdims=True)
    xc = x - m
    v = jnp.mean(xc * xc, axis=-1, keepdims=True)
    return xc * lax.rsqrt(v + 1e-5)


def _phi(t):
    return jnp.where(t > 0, t + 1.0, jnp.exp(t)) + 1e-6


def _gelu(x):
    c = 0.7978845608028654
    inner = x * (c + (c * 0.044715) * (x * x))
    hx = 0.5 * x
    return hx + hx * jnp.tanh(inner)


def _rows(i):
    if isinstance(i, int):
        return pl.ds(i * TM, TM)
    return pl.ds(pl.multiple_of(i * TM, TM), TM)


def _kernel(x_hbm, wqkv_hbm, wo_hbm, win_hbm, wsp_hbm, b_hbm, wout_hbm, out_hbm,
            x_v, wqkv_v, wo_v, win_v, wsp_v, b_v, wout_v, out_v,
            xa_s, xb_s, pq_s, h_s, z1_s, z2_s, kv_s, zs_s, zb_s, kvwo_s, bcol_s, zg_s, sems, xsems, osems):
    def x_copy(i):
        return pltpu.make_async_copy(x_hbm.at[_rows(i), :], x_v.at[_rows(i), :], xsems.at[i])

    def wqkv_copy(j):
        return pltpu.make_async_copy(wqkv_hbm.at[:, pl.ds(j * D, D)], wqkv_v.at[:, pl.ds(j * D, D)], sems.at[7 + j])

    c_wo = pltpu.make_async_copy(wo_hbm, wo_v, sems.at[2])
    c_win = pltpu.make_async_copy(win_hbm, win_v, sems.at[3])
    c_wsp = pltpu.make_async_copy(wsp_hbm, wsp_v, sems.at[4])
    c_b = pltpu.make_async_copy(b_hbm, b_v, sems.at[5])
    c_wout = pltpu.make_async_copy(wout_hbm, wout_v, sems.at[6])
    x_copy(0).start()
    wqkv_copy(1).start()

    kv_s[...] = jnp.zeros_like(kv_s)
    zs_s[...] = jnp.zeros_like(zs_s)

    def p1a(i, buf):
        x = x_v[_rows(i), :].astype(F32)
        buf[...] = _ln(x).astype(BF16)

    def p1_kv(pk, v):
        zs_s[...] += jnp.sum(pk, axis=0, keepdims=True)
        pkb = pk.astype(BF16)
        for j in range(4):
            kv_s[j] += lax.dot_general(
                pkb[:, j * 128:(j + 1) * 128], v[:, j * 128:(j + 1) * 128],
                (((0,), (0,)), ((), ())), preferred_element_type=F32)

    def p1b(i, buf):
        xn = buf[...]
        k = jnp.dot(xn, wqkv_v[:, D:2 * D], preferred_element_type=F32)
        v = jnp.dot(xn, wqkv_v[:, 2 * D:], preferred_element_type=F32).astype(BF16)
        q = jnp.dot(xn, wqkv_v[:, :D], preferred_element_type=F32)
        p1_kv(_phi(k), v)
        pq_s[_rows(i), :] = _phi(q).astype(BF16)

    x_copy(0).wait()
    wqkv_copy(2).start()
    p1a(0, xa_s)
    wqkv_copy(1).wait()
    wqkv_copy(0).start()
    x_copy(1).start()
    k0 = jnp.dot(xa_s[...], wqkv_v[:, D:2 * D], preferred_element_type=F32)
    pk0 = _phi(k0)
    wqkv_copy(2).wait()
    x_copy(2).start()
    x_copy(3).start()
    v0 = jnp.dot(xa_s[...], wqkv_v[:, 2 * D:], preferred_element_type=F32).astype(BF16)
    wqkv_copy(0).wait()
    x_copy(1).wait()
    for i in range(4, NB):
        x_copy(i).start()
    q0 = jnp.dot(xa_s[...], wqkv_v[:, :D], preferred_element_type=F32)
    p1a(1, xb_s)
    p1_kv(pk0, v0)
    pq_s[_rows(0), :] = _phi(q0).astype(BF16)
    c_b.start()
    c_wo.start()
    c_win.start()
    c_wout.start()
    c_wsp.start()

    def p1(j, c):
        x_copy(2 * j + 2).wait()
        x_copy(2 * j + 3).wait()
        p1a(2 * j + 2, xa_s)
        p1b(2 * j + 1, xb_s)
        p1a(2 * j + 3, xb_s)
        p1b(2 * j + 2, xa_s)
        return c

    lax.fori_loop(0, NB // 2 - 1, p1, 0)
    c_wo.wait()
    c_b.wait()
    k7 = jnp.dot(xb_s[...], wqkv_v[:, D:2 * D], preferred_element_type=F32)
    v7 = jnp.dot(xb_s[...], wqkv_v[:, 2 * D:], preferred_element_type=F32).astype(BF16)
    p1_kv(_phi(k7), v7)
    pq_s[_rows(NB - 1), :D // 2] = _phi(
        jnp.dot(xb_s[...], wqkv_v[:, :D // 2], preferred_element_type=F32)).astype(BF16)

    rr = lax.broadcasted_iota(jnp.int32, (128, 128), 0) // DH
    cc = lax.broadcasted_iota(jnp.int32, (128, 128), 1) // DH
    mask = rr == cc
    for j in range(4):
        kvm = jnp.where(mask, kv_s[j], 0.0).astype(BF16)
        kvwo_s[j * 128:(j + 1) * 128, :] = jnp.dot(
            kvm, wo_v[j * 128:(j + 1) * 128, :], preferred_element_type=F32).astype(BF16)
        zrow = jnp.broadcast_to(zs_s[:, j * 128:(j + 1) * 128], (128, 128))
        zb_s[j] = jnp.where(mask, zrow.T, 0.0).astype(BF16)
    bb = b_v[...].astype(F32)
    for j in range(16):
        bcol_s[j * 128:(j + 1) * 128, :] = jnp.broadcast_to(bb[j:j + 1, :], (128, 128)).T

    def p2a1(i):
        pq = pq_s[_rows(i), :]
        den = jnp.concatenate(
            [jnp.dot(pq[:, j * 128:(j + 1) * 128], zb_s[j], preferred_element_type=F32)
             for j in range(4)], axis=1) + 1e-6
        return (pq.astype(F32) * pl.reciprocal(den, approx=True)).astype(BF16)

    def p2a2(i, a, buf):
        h = x_v[_rows(i), :].astype(F32) + jnp.dot(a, kvwo_s[...], preferred_element_type=F32)
        h_s[_rows(i), :] = h
        buf[...] = _ln(h).astype(BF16)

    def p2b1(i, buf):
        zg_s[...] = _gelu(jnp.dot(buf[...], win_v[:, FH:], preferred_element_type=F32))
        z2_s[_rows(i), :] = _ln(zg_s[...]).astype(BF16)

    def p2b2(i, buf):
        z1_s[_rows(i), :] = _gelu(jnp.dot(buf[...], win_v[:, :FH], preferred_element_type=F32))

    def p2ab(ia, bufa, ib, bufb):
        a = p2a1(ia)
        p2b1(ib, bufb)
        p2a2(ia, a, bufa)
        p2b2(ib, bufb)

    a0 = p2a1(0)
    h0 = x_v[_rows(0), :].astype(F32) + jnp.dot(a0, kvwo_s[...], preferred_element_type=F32)
    h_s[_rows(0), :] = h0
    pq_s[_rows(NB - 1), D // 2:] = _phi(
        jnp.dot(xb_s[...], wqkv_v[:, D // 2:D], preferred_element_type=F32)).astype(BF16)
    xa_s[...] = _ln(h0).astype(BF16)
    c_win.wait()

    def p2(j, c):
        p2ab(2 * j + 1, xb_s, 2 * j, xa_s)
        p2ab(2 * j + 2, xa_s, 2 * j + 1, xb_s)
        return c

    lax.fori_loop(0, NB // 2 - 1, p2, 0)
    p2ab(NB - 1, xb_s, NB - 2, xa_s)
    p2b1(NB - 1, xb_s)
    p2b2(NB - 1, xb_s)

    c_wsp.wait()
    c_wout.wait()

    TM3 = 512
    def _rows3(i):
        if isinstance(i, int):
            return pl.ds(i * TM3, TM3)
        return pl.ds(pl.multiple_of(i * TM3, TM3), TM3)

    NSUB = 4
    SZ = TM3 // NSUB

    def out_copy(i, n):
        if isinstance(i, int):
            rs = pl.ds(i * TM3 + n * SZ, SZ)
        else:
            rs = pl.ds(pl.multiple_of(i * TM3 + n * SZ, SZ), SZ)
        return rs, pltpu.make_async_copy(out_v.at[rs, :], out_hbm.at[rs, :], osems.at[i * NSUB + n])

    def p3(i, c):
        g = jnp.dot(wsp_v[_rows3(i), :], z2_s[...], preferred_element_type=F32)
        bc = bcol_s[_rows3(i), :]
        g = g + jnp.concatenate([bc] * (FH // 128), axis=1)
        u = (z1_s[_rows3(i), :] * g).astype(BF16)
        for n in range(NSUB):
            rs, cp = out_copy(i, n)
            o = h_s[rs, :] + jnp.dot(u[n * SZ:(n + 1) * SZ, :], wout_v[...], preferred_element_type=F32)
            out_v[rs, :] = o.astype(BF16)
            cp.start()
        return c

    lax.fori_loop(0, S // TM3, p3, 0)
    for i in range(S // TM3):
        for n in range(NSUB):
            out_copy(i, n)[1].wait()


@jax.jit
def pallas_sequential_preLN__linear_attn_block__mixer_gmlp__prompt_kernel(
    A_x, A_wqkv, A_wo, B_x, B_w_in, B_w_sp, B_b_sp, B_w_out):
    x = A_x.reshape(S, D)
    b2 = B_b_sp.reshape(S // 128, 128)
    any_spec = pl.BlockSpec(memory_space=pl.ANY)
    out = pl.pallas_call(
        _kernel,
        out_shape=jax.ShapeDtypeStruct((S, D), BF16),
        in_specs=[any_spec] * 7,
        out_specs=any_spec,
        scratch_shapes=[
            pltpu.VMEM((S, D), BF16),
            pltpu.VMEM((D, 3 * D), BF16),
            pltpu.VMEM((D, D), BF16),
            pltpu.VMEM((D, 2 * FH), BF16),
            pltpu.VMEM((S, S), BF16),
            pltpu.VMEM((S // 128, 128), BF16),
            pltpu.VMEM((FH, D), BF16),
            pltpu.VMEM((S, D), BF16),
            pltpu.VMEM((TM, D), BF16),
            pltpu.VMEM((TM, D), BF16),
            pltpu.VMEM((S, D), BF16),
            pltpu.VMEM((S, D), F32),
            pltpu.VMEM((S, FH), F32),
            pltpu.VMEM((S, FH), BF16),
            pltpu.VMEM((4, 128, 128), F32),
            pltpu.VMEM((1, D), F32),
            pltpu.VMEM((4, 128, 128), BF16),
            pltpu.VMEM((D, D), BF16),
            pltpu.VMEM((S, 128), F32),
            pltpu.VMEM((TM, FH), F32),
            pltpu.SemaphoreType.DMA((10,)),
            pltpu.SemaphoreType.DMA((NB,)),
            pltpu.SemaphoreType.DMA((16,)),
        ],
        compiler_params=pltpu.CompilerParams(vmem_limit_bytes=100 * 1024 * 1024),
    )(x, A_wqkv, A_wo, B_w_in, B_w_sp, b2, B_w_out)
    return out.reshape(1, S, D)
```

```python
import jax
import jax.numpy as jnp
from jax import lax
import jax.experimental.pallas as pl
import jax.experimental.pallas.tpu as pltpu

S = 2048
D = 512
FH = 896
DH = 16
TM = 256
NB = S // TM
TM3 = 512
NSUB = 4
SZ3 = TM3 // NSUB
LN_EPS = 1e-5
F32 = jnp.float32
BF16 = jnp.bfloat16


def _ln(x):
    m = jnp.mean(x, axis=-1, keepdims=True)
    xc = x - m
    v = jnp.mean(xc * xc, axis=-1, keepdims=True)
    return xc * lax.rsqrt(v + LN_EPS)


def _phi(t):
    return jnp.where(t > 0, t + 1.0, jnp.exp(t)) + 1e-6


def _gelu(x):
    c = 0.7978845608028654
    inner = x * (c + (c * 0.044715) * (x * x))
    hx = 0.5 * x
    return hx + hx * jnp.tanh(inner)


def _dot(a, b):
    return jnp.dot(a, b, preferred_element_type=F32)


def _ds(i, stride, off, size):
    if isinstance(i, int):
        return pl.ds(i * stride + off, size)
    return pl.ds(pl.multiple_of(i * stride + off, size), size)


def _rows(i):
    return _ds(i, TM, 0, TM)


def _kernel(x_hbm, wqkv_hbm, wo_hbm, win_hbm, wsp_hbm, b_hbm, wout_hbm, out_hbm,
            x_v, wqkv_v, wo_v, win_v, wsp_v, b_v, wout_v, out_v,
            xa_s, xb_s, pq_s, h_s, z1_s, z2_s, kv_s, zs_s, zb_s, kvwo_s, bcol_s, zg_s,
            sems, xsems, osems):
    def x_copy(i):
        return pltpu.make_async_copy(x_hbm.at[_rows(i), :], x_v.at[_rows(i), :], xsems.at[i])

    def wqkv_copy(j):
        return pltpu.make_async_copy(wqkv_hbm.at[:, pl.ds(j * D, D)],
                                     wqkv_v.at[:, pl.ds(j * D, D)], sems.at[5 + j])

    c_wo = pltpu.make_async_copy(wo_hbm, wo_v, sems.at[0])
    c_win = pltpu.make_async_copy(win_hbm, win_v, sems.at[1])
    c_wsp = pltpu.make_async_copy(wsp_hbm, wsp_v, sems.at[2])
    c_b = pltpu.make_async_copy(b_hbm, b_v, sems.at[3])
    c_wout = pltpu.make_async_copy(wout_hbm, wout_v, sems.at[4])
    x_copy(0).start()
    wqkv_copy(1).start()

    kv_s[...] = jnp.zeros_like(kv_s)
    zs_s[...] = jnp.zeros_like(zs_s)

    def p1_ln(i, buf):
        buf[...] = _ln(x_v[_rows(i), :].astype(F32)).astype(BF16)

    def p1_kv(pk, v):
        zs_s[...] += jnp.sum(pk, axis=0, keepdims=True)
        pkb = pk.astype(BF16)
        for j in range(4):
            kv_s[j] += lax.dot_general(
                pkb[:, j * 128:(j + 1) * 128], v[:, j * 128:(j + 1) * 128],
                (((0,), (0,)), ((), ())), preferred_element_type=F32)

    def p1_mm(i, buf):
        xn = buf[...]
        k = _dot(xn, wqkv_v[:, D:2 * D])
        v = _dot(xn, wqkv_v[:, 2 * D:]).astype(BF16)
        q = _dot(xn, wqkv_v[:, :D])
        p1_kv(_phi(k), v)
        pq_s[_rows(i), :] = _phi(q).astype(BF16)

    x_copy(0).wait()
    wqkv_copy(2).start()
    p1_ln(0, xa_s)
    wqkv_copy(1).wait()
    wqkv_copy(0).start()
    x_copy(1).start()
    pk0 = _phi(_dot(xa_s[...], wqkv_v[:, D:2 * D]))
    wqkv_copy(2).wait()
    x_copy(2).start()
    x_copy(3).start()
    v0 = _dot(xa_s[...], wqkv_v[:, 2 * D:]).astype(BF16)
    wqkv_copy(0).wait()
    x_copy(1).wait()
    for i in range(4, NB):
        x_copy(i).start()
    q0 = _dot(xa_s[...], wqkv_v[:, :D])
    p1_ln(1, xb_s)
    p1_kv(pk0, v0)
    pq_s[_rows(0), :] = _phi(q0).astype(BF16)
    c_b.start()
    c_wo.start()
    c_win.start()
    c_wout.start()
    c_wsp.start()

    def p1(j, c):
        x_copy(2 * j + 2).wait()
        x_copy(2 * j + 3).wait()
        p1_ln(2 * j + 2, xa_s)
        p1_mm(2 * j + 1, xb_s)
        p1_ln(2 * j + 3, xb_s)
        p1_mm(2 * j + 2, xa_s)
        return c

    lax.fori_loop(0, NB // 2 - 1, p1, 0)
    c_wo.wait()
    c_b.wait()

    k7 = _dot(xb_s[...], wqkv_v[:, D:2 * D])
    v7 = _dot(xb_s[...], wqkv_v[:, 2 * D:]).astype(BF16)
    p1_kv(_phi(k7), v7)
    pq_s[_rows(NB - 1), :D // 2] = _phi(_dot(xb_s[...], wqkv_v[:, :D // 2])).astype(BF16)

    rr = lax.broadcasted_iota(jnp.int32, (128, 128), 0) // DH
    cc = lax.broadcasted_iota(jnp.int32, (128, 128), 1) // DH
    same_head = rr == cc
    for j in range(4):
        kvm = jnp.where(same_head, kv_s[j], 0.0).astype(BF16)
        kvwo_s[j * 128:(j + 1) * 128, :] = _dot(kvm, wo_v[j * 128:(j + 1) * 128, :]).astype(BF16)
        zrow = jnp.broadcast_to(zs_s[:, j * 128:(j + 1) * 128], (128, 128))
        zb_s[j] = jnp.where(same_head, zrow.T, 0.0).astype(BF16)
    bb = b_v[...].astype(F32)
    for j in range(S // 128):
        bcol_s[j * 128:(j + 1) * 128, :] = jnp.broadcast_to(bb[j:j + 1, :], (128, 128)).T

    HM = TM // 2

    def p2_scale(i):
        pq = pq_s[_rows(i), :]
        den = jnp.concatenate(
            [_dot(pq[:, j * 128:(j + 1) * 128], zb_s[j]) for j in range(4)], axis=1) + 1e-6
        return (pq.astype(F32) * pl.reciprocal(den, approx=True)).astype(BF16)

    def p2_attn(i, a, buf, r):
        rows = _ds(i, TM, r * HM, HM)
        h = x_v[rows, :].astype(F32) + _dot(a[r * HM:(r + 1) * HM, :], kvwo_s[...])
        h_s[rows, :] = h
        buf[r * HM:(r + 1) * HM, :] = _ln(h).astype(BF16)

    def p2_z2(i, buf, r):
        rows = _ds(i, TM, r * HM, HM)
        zg_s[r * HM:(r + 1) * HM, :] = _gelu(_dot(buf[r * HM:(r + 1) * HM, :], win_v[:, FH:]))
        zz = zg_s[r * HM:(r + 1) * HM, :]
        m = jnp.mean(zz, axis=-1, keepdims=True)
        xc = zz - m
        rs = lax.rsqrt(jnp.mean(xc * xc, axis=-1, keepdims=True) + LN_EPS)
        for t in range(FH // 128):
            z2_s[rows, t * 128:(t + 1) * 128] = (
                (zg_s[r * HM:(r + 1) * HM, t * 128:(t + 1) * 128] - m) * rs).astype(BF16)

    def p2_z1(i, buf):
        z1_s[_rows(i), :] = _dot(buf[...], win_v[:, :FH])

    def p2_pair(ia, bufa, ib, bufb):
        a = p2_scale(ia)
        p2_z2(ib, bufb, 0)
        p2_attn(ia, a, bufa, 0)
        p2_z2(ib, bufb, 1)
        p2_attn(ia, a, bufa, 1)
        p2_z1(ib, bufb)

    a0 = p2_scale(0)
    h0 = x_v[_rows(0), :].astype(F32) + _dot(a0, kvwo_s[...])
    h_s[_rows(0), :] = h0
    pq_s[_rows(NB - 1), D // 2:] = _phi(_dot(xb_s[...], wqkv_v[:, D // 2:D])).astype(BF16)
    xa_s[...] = _ln(h0).astype(BF16)
    c_win.wait()

    def p2(j, c):
        p2_pair(2 * j + 1, xb_s, 2 * j, xa_s)
        p2_pair(2 * j + 2, xa_s, 2 * j + 1, xb_s)
        return c

    lax.fori_loop(0, NB // 2 - 1, p2, 0)
    p2_pair(NB - 1, xb_s, NB - 2, xa_s)
    p2_z2(NB - 1, xb_s, 0)
    p2_z2(NB - 1, xb_s, 1)
    p2_z1(NB - 1, xb_s)

    c_wsp.wait()
    c_wout.wait()

    def out_copy(i, n):
        rows = _ds(i, TM3, n * SZ3, SZ3)
        return rows, pltpu.make_async_copy(out_v.at[rows, :], out_hbm.at[rows, :],
                                           osems.at[i * NSUB + n])

    def p3(i, c):
        rows3 = _ds(i, TM3, 0, TM3)
        g = _dot(wsp_v[rows3, :], z2_s[...])
        g = g + jnp.concatenate([bcol_s[rows3, :]] * (FH // 128), axis=1)
        u = (_gelu(z1_s[rows3, :]) * g).astype(BF16)
        for n in range(NSUB):
            rows, cp = out_copy(i, n)
            o = h_s[rows, :] + _dot(u[n * SZ3:(n + 1) * SZ3, :], wout_v[...])
            out_v[rows, :] = o.astype(BF16)
            cp.start()
        return c

    lax.fori_loop(0, S // TM3, p3, 0)
    for i in range(S // TM3):
        for n in range(NSUB):
            out_copy(i, n)[1].wait()


@jax.jit
def pallas_sequential_preLN__linear_attn_block__mixer_gmlp__prompt_kernel(
    A_x: jax.Array,
    A_wqkv: jax.Array,
    A_wo: jax.Array,
    B_x: jax.Array,
    B_w_in: jax.Array,
    B_w_sp: jax.Array,
    B_b_sp: jax.Array,
    B_w_out: jax.Array,
):
    del B_x
    x = A_x.reshape(S, D)
    b2 = B_b_sp.reshape(S // 128, 128)
    any_spec = pl.BlockSpec(memory_space=pl.ANY)
    out = pl.pallas_call(
        _kernel,
        out_shape=jax.ShapeDtypeStruct((S, D), BF16),
        in_specs=[any_spec] * 7,
        out_specs=any_spec,
        scratch_shapes=[
            pltpu.VMEM((S, D), BF16),
            pltpu.VMEM((D, 3 * D), BF16),
            pltpu.VMEM((D, D), BF16),
            pltpu.VMEM((D, 2 * FH), BF16),
            pltpu.VMEM((S, S), BF16),
            pltpu.VMEM((S // 128, 128), BF16),
            pltpu.VMEM((FH, D), BF16),
            pltpu.VMEM((S, D), BF16),
            pltpu.VMEM((TM, D), BF16),
            pltpu.VMEM((TM, D), BF16),
            pltpu.VMEM((S, D), BF16),
            pltpu.VMEM((S, D), F32),
            pltpu.VMEM((S, FH), F32),
            pltpu.VMEM((S, FH), BF16),
            pltpu.VMEM((4, 128, 128), F32),
            pltpu.VMEM((1, D), F32),
            pltpu.VMEM((4, 128, 128), BF16),
            pltpu.VMEM((D, D), BF16),
            pltpu.VMEM((S, 128), F32),
            pltpu.VMEM((TM, FH), F32),
            pltpu.SemaphoreType.DMA((8,)),
            pltpu.SemaphoreType.DMA((NB,)),
            pltpu.SemaphoreType.DMA((S // TM3 * NSUB,)),
        ],
        compiler_params=pltpu.CompilerParams(vmem_limit_bytes=100 * 1024 * 1024),
    )(x, A_wqkv, A_wo, B_w_in, B_w_sp, b2, B_w_out)
    return out.reshape(1, S, D)
```
